```python
import os as _os
_os.environ.setdefault("JAX_PLATFORMS", "cpu")
import jax
import jax.numpy as jnp

def _softmax(x, axis=-1):
    return jax.nn.softmax(x, axis=axis)
def _gelu(x):
    return jax.nn.gelu(x, approximate=True)
def _silu(x):
    return jax.nn.silu(x)
def _sigmoid(x):
    return jax.nn.sigmoid(x)
def _layernorm(x, axis=-1, eps=1e-5):
    m = jnp.mean(x, axis=axis, keepdims=True)
    v = jnp.var(x, axis=axis, keepdims=True)
    return (x - m) / jnp.sqrt(v + eps)
def _scatter_add(tgt, idx, src, axis=0):
    return tgt.at[idx].add(src)
def _segment_sum(src, seg, n):
    return jax.ops.segment_sum(src, seg, n)
class _Rng:
    def __init__(self, key):
        self._k = key
    def _next(self):
        self._k, sub = jax.random.split(self._k)
        return sub
    def normal(self, shape):
        return jax.random.normal(self._next(), shape, dtype=jnp.bfloat16)
    def randint(self, lo, hi, shape):
        return jax.random.randint(self._next(), shape, lo, hi, dtype=jnp.int32)
    def uniform(self, shape, lo=0.0, hi=1.0):
        return jax.random.uniform(self._next(), shape, jnp.bfloat16, lo, hi)
    def permutation(self, n):
        return jax.random.permutation(self._next(), n)


kernel_name = 'concat_heads__mha_block_cached__gqa_block_cached__near_ridge'

def setup_inputs():
    _rng = _Rng(jax.random.key(int.from_bytes(__import__("os").urandom(4), "little")))
    _w = (lambda a: (lambda t: t.astype(jnp.bfloat16) if jnp.issubdtype(t.dtype, jnp.floating) else t)(jnp.asarray(a)))
    def _A_setup():
        B, Sq, D = 16, 48, 1024
        H, Sk, Dh = 32, 48, 128
        return {
            "x": _w((lambda *s: _rng.normal(s) * 0.8)(B, Sq, D)),
            "k_cache": _w((lambda *s: _rng.normal(s) * 0.8)(B, H, Sk, Dh)),
            "v_cache": _w((lambda *s: _rng.normal(s) * 0.05)(B, H, Sk, Dh)),
            "wq": _w((lambda *s: _rng.normal(s) * 0.8)(D, H * Dh) * (D ** -0.5)),
            "wo": _w((lambda *s: _rng.normal(s) * 0.05)(H * Dh, D) * ((H * Dh) ** -0.5)),
        }
    _A_in = _A_setup()

    def _B_setup():
        B, Sq, D = 16, 48, 1024
        Hq, Hkv, Sk, Dh = 32, 32, 48, 128
        assert Hq % Hkv == 0, (Hq, Hkv)
        return {
            "x": _w((lambda *s: _rng.normal(s) * 0.8)(B, Sq, D)),
            "k_cache": _w((lambda *s: _rng.normal(s) * 0.8)(B, Hkv, Sk, Dh)),
            "v_cache": _w((lambda *s: _rng.normal(s) * 0.05)(B, Hkv, Sk, Dh)),
            "wq": _w((lambda *s: _rng.normal(s) * 0.8)(D, Hq * Dh) * (D ** -0.5)),
            "wo": _w((lambda *s: _rng.normal(s) * 0.05)(Hq * Dh, D) * ((Hq * Dh) ** -0.5)),
        }
    _B_in = _B_setup()

    return {
        "A_x": _A_in["x"],
        "A_k_cache": _A_in["k_cache"],
        "A_v_cache": _A_in["v_cache"],
        "A_wq": _A_in["wq"],
        "A_wo": _A_in["wo"],
        "B_x": _B_in["x"],
        "B_k_cache": _B_in["k_cache"],
        "B_v_cache": _B_in["v_cache"],
        "B_wq": _B_in["wq"],
        "B_wo": _B_in["wo"],
    }

def reference(A_x, A_k_cache, A_v_cache, A_wq, A_wo, B_x, B_k_cache, B_v_cache, B_wq, B_wo):
    def _A_ref(x, k_cache, v_cache, wq, wo):
        B, Sq, D = x.shape
        H, Dh = 32, 128
        q = (lambda x, *d: x.transpose(*d))((x @ wq).reshape(B, Sq, H, Dh), 0, 2, 1, 3)
        scores = jnp.einsum("bhqd,bhkd->bhqk", q, k_cache) * (Dh ** -0.5)
        p = _softmax(scores, axis=-1)
        o = jnp.einsum("bhqk,bhkd->bhqd", p, v_cache)
        return (lambda x, *d: x.transpose(*d))(o, 0, 2, 1, 3).reshape(B, Sq, H * Dh) @ wo

    def _B_ref(x, k_cache, v_cache, wq, wo):
        B, Sq, D = x.shape
        Hq, Dh = 32, 128
        Hkv = k_cache.shape[1]
        rep = Hq // Hkv
        q = (lambda x, *d: x.transpose(*d))((x @ wq).reshape(B, Sq, Hq, Dh), 0, 2, 1, 3)
        k = jnp.repeat(k_cache, rep, axis=1)
        v = jnp.repeat(v_cache, rep, axis=1)
        scores = jnp.einsum("bhqd,bhkd->bhqk", q, k) * (Dh ** -0.5)
        p = _softmax(scores, axis=-1)
        o = jnp.einsum("bhqk,bhkd->bhqd", p, v)
        return (lambda x, *d: x.transpose(*d))(o, 0, 2, 1, 3).reshape(B, Sq, Hq * Dh) @ wo

    a = _A_ref(A_x, A_k_cache, A_v_cache, A_wq, A_wo)
    b = _B_ref(B_x, B_k_cache, B_v_cache, B_wq, B_wo)
    return jnp.concatenate([a, b], axis=-1)
```

```python
import math

import jax
import jax.numpy as jnp
from jax import lax
import jax.experimental.pallas as pl
import jax.experimental.pallas.tpu as pltpu


@jax.jit
def pallas_concat_heads__mha_block_cached__gqa_block_cached__near_ridge_kernel(
    A_x: jax.Array,
    A_k_cache: jax.Array,
    A_v_cache: jax.Array,
    A_wq: jax.Array,
    A_wo: jax.Array,
    B_x: jax.Array,
    B_k_cache: jax.Array,
    B_v_cache: jax.Array,
    B_wq: jax.Array,
    B_wo: jax.Array,
):
    B, Sq, D = A_x.shape
    _, H, Sk, Dh = A_k_cache.shape
    assert B_k_cache.shape == A_k_cache.shape
    M = B * Sq
    bf, f32 = jnp.bfloat16, jnp.float32

    KCH = (128, 128, 256, 512)
    N0 = 8
    NQL = 2
    QL = (H - N0) // NQL
    HB = 16
    NIT = 2 * H // HB
    QB = H // NIT
    OG = 4
    NT = D // OG
    LAST = (384, 192, 192)
    NK = len(KCH)
    S_Q = NK
    S_M = S_Q + NQL
    S_OUT = S_M + NIT
    NSEM = S_OUT + 1
    c = (Dh ** -0.5) * math.log2(math.e)

    def kernel(ax, ak, av, awq, awo, bx, bk, bv, bwq, bwo, out_hbm,
               x_s, k_s, v_s, wq1_s, wq2_s, wqb_s, wo_s, q_s, o_s, acc_s, out_s,
               one_s, sems):
        srcs = ((ak, av, awo), (bk, bv, bwo))
        cp = pltpu.make_async_copy

        init = []
        k0 = 0
        for i, kc in enumerate(KCH):
            sl = pl.ds(k0, kc)
            init.append([
                cp(ax.at[:, sl], x_s.at[0, :, sl], sems.at[i]),
                cp(awq.at[sl, pl.ds(0, N0 * Dh)], wq1_s.at[sl, :], sems.at[i]),
            ])
            k0 += kc
            for d in init[i]:
                d.start()
        for j in range(NQL):
            cp(awq.at[:, pl.ds((N0 + j * QL) * Dh, QL * Dh)], wq2_s.at[j],
               sems.at[S_Q + j]).start()
        for it in range(NIT):
            br, hh = divmod(it * HB, H)
            sem = sems.at[S_M + it]
            if it == 0:
                cp(bx, x_s.at[1], sem).start()
            cp(srcs[br][0].at[:, pl.ds(hh, HB)], k_s.at[it], sem).start()
            cp(bwq.at[:, pl.ds(it * QB * Dh, QB * Dh)], wqb_s.at[it], sem).start()
            cp(srcs[br][1].at[:, pl.ds(hh, HB)], v_s.at[it], sem).start()
            cp(srcs[br][2].at[pl.ds(hh * Dh, HB * Dh), :], wo_s.at[it], sem).start()

        def put_q(first, t):
            for j in range(t.shape[1] // Dh):
                q_s[first + j] = t[:, j * Dh:(j + 1) * Dh]

        def qloop(j, carry):
            cp(wq2_s.at[j], wq2_s.at[j], sems.at[S_Q + j]).wait()
            q = jnp.dot(x_s[0], wq2_s[j], preferred_element_type=f32)
            put_q(N0 + j * QL, q.astype(bf))
            return carry

        def main(it, carry):
            br = lax.shift_right_logical(it, 1)
            second = (it & 1) == 1
            sem = sems.at[S_M + it]

            @pl.when(it == 0)
            def _():
                cp(bx, x_s.at[1], sem).wait()
            cp(k_s.at[it], k_s.at[it], sem).wait()
            cp(wqb_s.at[it], wqb_s.at[it], sem).wait()
            cp(v_s.at[it], v_s.at[it], sem).wait()
            cp(wo_s.at[it], wo_s.at[it], sem).wait()

            def oproj(g, j, r0=0, r1=M):
                cs = slice(j * NT, (j + 1) * NT)
                t = jnp.dot(o_s[g, r0:r1, :],
                            wo_s[it, g * OG * Dh:(g + 1) * OG * Dh, cs],
                            preferred_element_type=f32)
                prev = acc_s[r0:r1, cs]
                if g == 0:
                    prev = jnp.where(second, prev, 0.0)
                t = t + prev
                acc_s[r0:r1, cs] = t
                if g == HB // OG - 1:
                    out_s[br, r0:r1, cs] = t.astype(bf)

                    @pl.when(second)
                    def _():
                        col = pl.multiple_of(br * D + j * NT, NT)
                        cp(out_s.at[br, pl.ds(r0, r1 - r0), pl.ds(j * NT, NT)],
                           out_hbm.at[pl.ds(r0, r1 - r0), pl.ds(col, NT)],
                           sems.at[S_OUT]).start()

            for s in range(HB):
                qh = q_s[it * HB + s].reshape(B, Sq, Dh)
                sc = lax.dot_general(qh, k_s[it, :, s], (((2,), (2,)), ((0,), (0,))),
                                     preferred_element_type=f32)
                m = jnp.max(sc, axis=-1, keepdims=True)
                p = jnp.exp2((sc - m) * c)
                l = jnp.sum(p, axis=-1, keepdims=True)
                r = pl.reciprocal(l, approx=True)
                r = r * (2.0 - l * r)
                p = (p * r).astype(bf)
                if s < QB:
                    q_s[H + it * QB + s] = jnp.dot(
                        x_s[1], wqb_s[it, :, s * Dh:(s + 1) * Dh],
                        preferred_element_type=f32).astype(bf)
                if s >= OG:
                    oproj(s // OG - 1, s % OG)
                o = lax.dot_general(p, v_s[it, :, s], (((2,), (1,)), ((0,), (0,))),
                                    preferred_element_type=f32)
                o_s[s // OG, :, (s % OG) * Dh:(s % OG + 1) * Dh] = (
                    o.reshape(M, Dh).astype(bf))
            for j in range(OG - 1):
                oproj(HB // OG - 1, j)
            r0 = 0
            for rr in LAST:
                oproj(HB // OG - 1, OG - 1, r0, r0 + rr)
                r0 += rr
            return carry

        def everything(_, carry):
            k0 = 0
            for i, kc in enumerate(KCH):
                for d in init[i]:
                    d.wait()
                t = jnp.dot(x_s[0, :, k0:k0 + kc], wq1_s[k0:k0 + kc, :],
                            preferred_element_type=f32)
                if i == 0:
                    acc_s[...] = t
                elif i < NK - 1:
                    acc_s[...] += t
                else:
                    put_q(0, (acc_s[...] + t).astype(bf))
                k0 += kc
            lax.fori_loop(0, NQL, qloop, 0)
            lax.fori_loop(0, NIT, main, 0)
            cp(out_s, out_s, sems.at[S_OUT]).wait()
            return carry

        one_s[0] = 1
        lax.fori_loop(0, one_s[0], everything, 0)

    any_spec = pl.BlockSpec(memory_space=pl.ANY)
    out = pl.pallas_call(
        kernel,
        in_specs=[any_spec] * 10,
        out_specs=any_spec,
        out_shape=jax.ShapeDtypeStruct((M, 2 * D), bf),
        scratch_shapes=[
            pltpu.VMEM((2, M, D), bf),
            pltpu.VMEM((NIT, B, HB, Sk, Dh), bf),
            pltpu.VMEM((NIT, B, HB, Sk, Dh), bf),
            pltpu.VMEM((D, N0 * Dh), bf),
            pltpu.VMEM((NQL, D, QL * Dh), bf),
            pltpu.VMEM((NIT, D, QB * Dh), bf),
            pltpu.VMEM((NIT, HB * Dh, D), bf),
            pltpu.VMEM((2 * H, M, Dh), bf),
            pltpu.VMEM((HB // OG, M, OG * Dh), bf),
            pltpu.VMEM((M, D), f32),
            pltpu.VMEM((2, M, D), bf),
            pltpu.SMEM((1,), jnp.int32),
            pltpu.SemaphoreType.DMA((NSEM,)),
        ],
        compiler_params=pltpu.CompilerParams(
            vmem_limit_bytes=120 * 1024 * 1024,
            disable_bounds_checks=True,
            disable_semaphore_checks=True,
        ),
    )(A_x.reshape(M, D), A_k_cache, A_v_cache, A_wq, A_wo,
      B_x.reshape(M, D), B_k_cache, B_v_cache, B_wq, B_wo)
    return out.reshape(B, Sq, 2 * D)
```

```python
import math

import jax
import jax.numpy as jnp
from jax import lax
import jax.experimental.pallas as pl
import jax.experimental.pallas.tpu as pltpu


@jax.jit
def pallas_concat_heads__mha_block_cached__gqa_block_cached__near_ridge_kernel(
    A_x: jax.Array,
    A_k_cache: jax.Array,
    A_v_cache: jax.Array,
    A_wq: jax.Array,
    A_wo: jax.Array,
    B_x: jax.Array,
    B_k_cache: jax.Array,
    B_v_cache: jax.Array,
    B_wq: jax.Array,
    B_wo: jax.Array,
):
    B, Sq, D = A_x.shape
    _, H, Sk, Dh = A_k_cache.shape
    assert B_k_cache.shape == A_k_cache.shape
    M = B * Sq
    W = H * Dh
    bf, f32 = jnp.bfloat16, jnp.float32

    U = 128
    K0 = 2 * U
    NQL = 2
    KL = (D - K0) // NQL
    AR = 384
    C1, C2, C3 = 4 * Dh, 8 * Dh, 24 * Dh
    NS = 1024
    HB = 16
    NIT = 2 * H // HB
    QB = H // NIT
    OG = 4
    NT = D // OG
    LAST = (384, 192, 144, 48)
    S_Q = 4
    S_M = S_Q + NQL
    S_OUT = S_M + NIT
    NSEM = S_OUT + 1
    c = (Dh ** -0.5) * math.log2(math.e)

    def kernel(ax, ak, av, awq, awo, bx, bk, bv, bwq, bwo, out_hbm,
               x0_s, xk_s, xb_s, k_s, v_s, w0_s, wk_s, wqb_s, wo_s,
               q_s, o_s, qacc_s, acc_s, out_s, one_s, sems):
        srcs = ((ak, av, awo), (bk, bv, bwo))
        cp = pltpu.make_async_copy

        def cpx(r0, r1, k0, k1, sem):
            idx = (pl.ds(r0, r1 - r0), pl.ds(k0, k1 - k0))
            return cp(ax.at[idx], x0_s.at[idx], sem)

        def cpw(k0, k1, c0, c1, sem):
            idx = (pl.ds(k0, k1 - k0), pl.ds(c0, c1 - c0))
            return cp(awq.at[idx], w0_s.at[idx], sem)

        init = [
            [cpx(0, AR, 0, U, sems.at[0]), cpw(0, U, 0, C1, sems.at[0])],
            [cpx(AR, M, 0, U, sems.at[1]), cpw(0, U, C1, C2, sems.at[1])],
            [cpw(0, U, C2, C3, sems.at[2])],
            [cpw(0, U, C3, W, sems.at[3]), cpx(0, M, U, K0, sems.at[3]),
             cpw(U, K0, 0, W, sems.at[3])],
        ]
        for group in init:
            for d in group:
                d.start()
        for j in range(NQL):
            sl = pl.ds(K0 + j * KL, KL)
            cp(ax.at[:, sl], xk_s.at[j], sems.at[S_Q + j]).start()
            cp(awq.at[sl, :], wk_s.at[j], sems.at[S_Q + j]).start()
        for it in range(NIT):
            br, hh = divmod(it * HB, H)
            sem = sems.at[S_M + it]
            if it == 0:
                cp(bx, xb_s, sem).start()
            cp(srcs[br][0].at[:, pl.ds(hh, HB)], k_s.at[it], sem).start()
            cp(bwq.at[:, pl.ds(it * QB * Dh, QB * Dh)], wqb_s.at[it], sem).start()
            cp(srcs[br][1].at[:, pl.ds(hh, HB)], v_s.at[it], sem).start()
            cp(srcs[br][2].at[pl.ds(hh * Dh, HB * Dh), :], wo_s.at[it], sem).start()

        def wait(i):
            for d in init[i]:
                d.wait()

        def first(r0, r1, c0, c1):
            for a in range(c0, c1, NS):
                b = min(a + NS, c1)
                qacc_s[r0:r1, a:b] = jnp.dot(x0_s[r0:r1, 0:U], w0_s[0:U, a:b],
                                             preferred_element_type=f32)

        def qloop(j, carry):
            cp(xk_s.at[j], xk_s.at[j], sems.at[S_Q + j]).wait()
            cp(wk_s.at[j], wk_s.at[j], sems.at[S_Q + j]).wait()
            for a in range(0, W, NS):
                t = qacc_s[:, a:a + NS] + jnp.dot(xk_s[j], wk_s[j, :, a:a + NS],
                                                  preferred_element_type=f32)
                qacc_s[:, a:a + NS] = t
                t = t.astype(bf)
                for h in range(NS // Dh):
                    q_s[a // Dh + h] = t[:, h * Dh:(h + 1) * Dh]
            return carry

        def main(it, carry):
            br = lax.shift_right_logical(it, 1)
            second = (it & 1) == 1
            sem = sems.at[S_M + it]

            @pl.when(it == 0)
            def _():
                cp(bx, xb_s, sem).wait()
            cp(k_s.at[it], k_s.at[it], sem).wait()
            cp(wqb_s.at[it], wqb_s.at[it], sem).wait()
            cp(v_s.at[it], v_s.at[it], sem).wait()
            cp(wo_s.at[it], wo_s.at[it], sem).wait()

            def oproj(g, j, r0=0, r1=M):
                cs = slice(j * NT, (j + 1) * NT)
                t = jnp.dot(o_s[g, r0:r1, :],
                            wo_s[it, g * OG * Dh:(g + 1) * OG * Dh, cs],
                            preferred_element_type=f32)
                if g == 0:
                    prev = jnp.where(second, qacc_s[r0:r1, cs], 0.0)
                else:
                    prev = acc_s[r0:r1, cs]
                t = t + prev
                if g == HB // OG - 1:
                    qacc_s[r0:r1, cs] = t
                    out_s[br, r0:r1, cs] = t.astype(bf)

                    @pl.when(second)
                    def _():
                        col = pl.multiple_of(br * D + j * NT, NT)
                        cp(out_s.at[br, pl.ds(r0, r1 - r0), pl.ds(j * NT, NT)],
                           out_hbm.at[pl.ds(r0, r1 - r0), pl.ds(col, NT)],
                           sems.at[S_OUT]).start()
                else:
                    acc_s[r0:r1, cs] = t

            for s in range(HB):
                qh = q_s[it * HB + s].reshape(B, Sq, Dh)
                sc = lax.dot_general(qh, k_s[it, :, s], (((2,), (2,)), ((0,), (0,))),
                                     preferred_element_type=f32)
                m = jnp.max(sc, axis=-1, keepdims=True)
                p = jnp.exp2((sc - m) * c)
                l = jnp.sum(p, axis=-1, keepdims=True)
                r = pl.reciprocal(l, approx=True)
                r = r * (2.0 - l * r)
                p = (p * r).astype(bf)
                if s < QB:
                    q_s[H + it * QB + s] = jnp.dot(
                        xb_s[...], wqb_s[it, :, s * Dh:(s + 1) * Dh],
                        preferred_element_type=f32).astype(bf)
                if s >= OG:
                    oproj(s // OG - 1, s % OG)
                o = lax.dot_general(p, v_s[it, :, s], (((2,), (1,)), ((0,), (0,))),
                                    preferred_element_type=f32)
                o_s[s // OG, :, (s % OG) * Dh:(s % OG + 1) * Dh] = (
                    o.reshape(M, Dh).astype(bf))
            for j in range(OG - 1):
                oproj(HB // OG - 1, j)
            r0 = 0
            for rr in LAST:
                oproj(HB // OG - 1, OG - 1, r0, r0 + rr)
                r0 += rr
            return carry

        def everything(_, carry):
            wait(0)
            first(0, AR, 0, C1)
            wait(1)
            first(0, M, C1, C2)
            first(AR, M, 0, C1)
            wait(2)
            first(0, M, C2, C3)
            wait(3)
            for a in range(0, C3, NS):
                qacc_s[:, a:a + NS] += jnp.dot(x0_s[:, U:K0], w0_s[U:K0, a:a + NS],
                                               preferred_element_type=f32)
            qacc_s[:, C3:W] = jnp.dot(x0_s[...], w0_s[:, C3:W],
                                      preferred_element_type=f32)
            lax.fori_loop(0, NQL, qloop, 0)
            lax.fori_loop(0, NIT, main, 0)
            cp(out_s, out_s, sems.at[S_OUT]).wait()
            return carry

        one_s[0] = 1
        lax.fori_loop(0, one_s[0], everything, 0)

    any_spec = pl.BlockSpec(memory_space=pl.ANY)
    out = pl.pallas_call(
        kernel,
        in_specs=[any_spec] * 10,
        out_specs=any_spec,
        out_shape=jax.ShapeDtypeStruct((M, 2 * D), bf),
        scratch_shapes=[
            pltpu.VMEM((M, K0), bf),
            pltpu.VMEM((NQL, M, KL), bf),
            pltpu.VMEM((M, D), bf),
            pltpu.VMEM((NIT, B, HB, Sk, Dh), bf),
            pltpu.VMEM((NIT, B, HB, Sk, Dh), bf),
            pltpu.VMEM((K0, W), bf),
            pltpu.VMEM((NQL, KL, W), bf),
            pltpu.VMEM((NIT, D, QB * Dh), bf),
            pltpu.VMEM((NIT, HB * Dh, D), bf),
            pltpu.VMEM((2 * H, M, Dh), bf),
            pltpu.VMEM((HB // OG, M, OG * Dh), bf),
            pltpu.VMEM((M, W), f32),
            pltpu.VMEM((M, D), f32),
            pltpu.VMEM((2, M, D), bf),
            pltpu.SMEM((1,), jnp.int32),
            pltpu.SemaphoreType.DMA((NSEM,)),
        ],
        compiler_params=pltpu.CompilerParams(
            vmem_limit_bytes=124 * 1024 * 1024,
            disable_bounds_checks=True,
            disable_semaphore_checks=True,
        ),
    )(A_x.reshape(M, D), A_k_cache, A_v_cache, A_wq, A_wo,
      B_x.reshape(M, D), B_k_cache, B_v_cache, B_wq, B_wo)
    return out.reshape(B, Sq, 2 * D)
```

```python
import jax
import jax.numpy as jnp
import numpy as np
from jax import lax
import jax.experimental.pallas as pl
import jax.experimental.pallas.tpu as pltpu


@jax.jit
def pallas_concat_heads__mha_block_cached__gqa_block_cached__near_ridge_kernel(
    A_x: jax.Array,
    A_k_cache: jax.Array,
    A_v_cache: jax.Array,
    A_wq: jax.Array,
    A_wo: jax.Array,
    B_x: jax.Array,
    B_k_cache: jax.Array,
    B_v_cache: jax.Array,
    B_wq: jax.Array,
    B_wo: jax.Array,
):
    B, Sq, D = A_x.shape
    _, H, Sk, Dh = A_k_cache.shape
    assert B_k_cache.shape == A_k_cache.shape
    M = B * Sq
    W = H * Dh
    bf, f32 = jnp.bfloat16, jnp.float32

    U = 128
    K0 = 2 * U
    NQL = 2
    KL = (D - K0) // NQL
    AR = 384
    C1, C2, C3 = 4 * Dh, 8 * Dh, 24 * Dh
    HB = 16
    NIT = 2 * H // HB
    QB = H // NIT
    OG = 4
    NT = D // OG
    LAST = (384, 192, 144, 48)
    S_Q = 4
    S_M = S_Q + NQL
    S_OUT = S_M + NIT
    NSEM = S_OUT + 1
    scale = float(np.asarray(Dh ** -0.5, dtype=bf))

    def kernel(ax, ak, av, awq, awo, bx, bk, bv, bwq, bwo, out_hbm,
               x0_s, xk_s, xb_s, k_s, v_s, w0_s, wk_s, wqb_s, wo_s,
               q_s, o_s, qacc_s, acc_s, out_s, one_s, sems):
        srcs = ((ak, av, awo), (bk, bv, bwo))
        cp = pltpu.make_async_copy

        def cpx(r0, r1, k0, k1, sem):
            idx = (pl.ds(r0, r1 - r0), pl.ds(k0, k1 - k0))
            return cp(ax.at[idx], x0_s.at[idx], sem)

        def cpw(k0, k1, c0, c1, sem):
            idx = (pl.ds(k0, k1 - k0), pl.ds(c0, c1 - c0))
            return cp(awq.at[idx], w0_s.at[idx], sem)

        init = [
            [cpx(0, AR, 0, U, sems.at[0]), cpw(0, U, 0, C1, sems.at[0])],
            [cpx(AR, M, 0, U, sems.at[1]), cpw(0, U, C1, C2, sems.at[1])],
            [cpw(0, U, C2, C3, sems.at[2])],
            [cpw(0, U, C3, W, sems.at[3]), cpx(0, M, U, K0, sems.at[3]),
             cpw(U, K0, 0, W, sems.at[3])],
        ]
        for group in init:
            for d in group:
                d.start()

        def start_rest():
            for j in range(NQL):
                sl = pl.ds(K0 + j * KL, KL)
                cp(ax.at[:, sl], xk_s.at[j], sems.at[S_Q + j]).start()
                cp(awq.at[sl, :], wk_s.at[j], sems.at[S_Q + j]).start()
            for it in range(NIT):
                br, hh = divmod(it * HB, H)
                sem = sems.at[S_M + it]
                if it == 0:
                    cp(bx, xb_s, sem).start()
                cp(srcs[br][0].at[:, pl.ds(hh, HB)], k_s.at[it], sem).start()
                cp(bwq.at[:, pl.ds(it * QB * Dh, QB * Dh)], wqb_s.at[it], sem).start()
                cp(srcs[br][1].at[:, pl.ds(hh, HB)], v_s.at[it], sem).start()
                cp(srcs[br][2].at[pl.ds(hh * Dh, HB * Dh), :], wo_s.at[it], sem).start()

        def wait(i):
            for d in init[i]:
                d.wait()

        def first(r0, r1, c0, c1):
            qacc_s[r0:r1, c0:c1] = jnp.dot(x0_s[r0:r1, 0:U], w0_s[0:U, c0:c1],
                                           preferred_element_type=f32)

        def qloop(j, carry):
            cp(xk_s.at[j], xk_s.at[j], sems.at[S_Q + j]).wait()
            cp(wk_s.at[j], wk_s.at[j], sems.at[S_Q + j]).wait()
            t = qacc_s[...] + jnp.dot(xk_s[j], wk_s[j], preferred_element_type=f32)
            qacc_s[...] = t
            for h in range(H):
                q_s[h] = t[:, h * Dh:(h + 1) * Dh].astype(bf)
            return carry

        def main(it, carry):
            br = lax.shift_right_logical(it, 1)
            second = (it & 1) == 1
            sem = sems.at[S_M + it]

            @pl.when(it == 0)
            def _():
                cp(bx, xb_s, sem).wait()
            cp(k_s.at[it], k_s.at[it], sem).wait()
            cp(wqb_s.at[it], wqb_s.at[it], sem).wait()
            cp(v_s.at[it], v_s.at[it], sem).wait()
            cp(wo_s.at[it], wo_s.at[it], sem).wait()

            def oproj(g, j, r0=0, r1=M):
                cs = slice(j * NT, (j + 1) * NT)
                t = jnp.dot(o_s[g, r0:r1, :],
                            wo_s[it, g * OG * Dh:(g + 1) * OG * Dh, cs],
                            preferred_element_type=f32)
                if g == 0:
                    prev = jnp.where(second, qacc_s[r0:r1, cs], 0.0)
                else:
                    prev = acc_s[r0:r1, cs]
                t = t + prev
                if g == HB // OG - 1:
                    qacc_s[r0:r1, cs] = t
                    out_s[br, r0:r1, cs] = t.astype(bf)

                    @pl.when(second)
                    def _():
                        col = pl.multiple_of(br * D + j * NT, NT)
                        cp(out_s.at[br, pl.ds(r0, r1 - r0), pl.ds(j * NT, NT)],
                           out_hbm.at[pl.ds(r0, r1 - r0), pl.ds(col, NT)],
                           sems.at[S_OUT]).start()
                else:
                    acc_s[r0:r1, cs] = t

            for s in range(HB):
                qh = q_s[it * HB + s].reshape(B, Sq, Dh)
                sc = lax.dot_general(qh, k_s[it, :, s], (((2,), (2,)), ((0,), (0,))),
                                     preferred_element_type=f32)
                sc = sc.astype(bf).astype(f32)
                sc = (sc * scale).astype(bf).astype(f32)
                m = jnp.max(sc, axis=-1, keepdims=True)
                p = jnp.exp(sc - m)
                l = jnp.sum(p, axis=-1, keepdims=True)
                r = pl.reciprocal(l, approx=True)
                r = r * (2.0 - l * r)
                p = (p * r).astype(bf)
                if s < QB:
                    q_s[H + it * QB + s] = jnp.dot(
                        xb_s[...], wqb_s[it, :, s * Dh:(s + 1) * Dh],
                        preferred_element_type=f32).astype(bf)
                if s >= OG:
                    oproj(s // OG - 1, s % OG)
                o = lax.dot_general(p, v_s[it, :, s], (((2,), (1,)), ((0,), (0,))),
                                    preferred_element_type=f32)
                o_s[s // OG, :, (s % OG) * Dh:(s % OG + 1) * Dh] = (
                    o.reshape(M, Dh).astype(bf))
            for j in range(OG - 1):
                oproj(HB // OG - 1, j)
            r0 = 0
            for rr in LAST:
                oproj(HB // OG - 1, OG - 1, r0, r0 + rr)
                r0 += rr
            return carry

        def everything(_, carry):
            wait(0)
            start_rest()
            first(0, AR, 0, C1)
            wait(1)
            first(0, M, C1, C2)
            first(AR, M, 0, C1)
            wait(2)
            first(0, M, C2, C3)
            wait(3)
            qacc_s[:, 0:C3] += jnp.dot(x0_s[:, U:K0], w0_s[U:K0, 0:C3],
                                       preferred_element_type=f32)
            qacc_s[:, C3:W] = jnp.dot(x0_s[...], w0_s[:, C3:W],
                                      preferred_element_type=f32)
            lax.fori_loop(0, NQL, qloop, 0)
            lax.fori_loop(0, NIT, main, 0)
            cp(out_s, out_s, sems.at[S_OUT]).wait()
            return carry

        one_s[0] = 1
        lax.fori_loop(0, one_s[0], everything, 0)

    any_spec = pl.BlockSpec(memory_space=pl.ANY)
    out = pl.pallas_call(
        kernel,
        in_specs=[any_spec] * 10,
        out_specs=any_spec,
        out_shape=jax.ShapeDtypeStruct((M, 2 * D), bf),
        scratch_shapes=[
            pltpu.VMEM((M, K0), bf),
            pltpu.VMEM((NQL, M, KL), bf),
            pltpu.VMEM((M, D), bf),
            pltpu.VMEM((NIT, B, HB, Sk, Dh), bf),
            pltpu.VMEM((NIT, B, HB, Sk, Dh), bf),
            pltpu.VMEM((K0, W), bf),
            pltpu.VMEM((NQL, KL, W), bf),
            pltpu.VMEM((NIT, D, QB * Dh), bf),
            pltpu.VMEM((NIT, HB * Dh, D), bf),
            pltpu.VMEM((2 * H, M, Dh), bf),
            pltpu.VMEM((HB // OG, M, OG * Dh), bf),
            pltpu.VMEM((M, W), f32),
            pltpu.VMEM((M, D), f32),
            pltpu.VMEM((2, M, D), bf),
            pltpu.SMEM((1,), jnp.int32),
            pltpu.SemaphoreType.DMA((NSEM,)),
        ],
        compiler_params=pltpu.CompilerParams(
            vmem_limit_bytes=124 * 1024 * 1024,
            disable_bounds_checks=True,
            disable_semaphore_checks=True,
        ),
    )(A_x.reshape(M, D), A_k_cache, A_v_cache, A_wq, A_wo,
      B_x.reshape(M, D), B_k_cache, B_v_cache, B_wq, B_wo)
    return out.reshape(B, Sq, 2 * D)
```
